```python
import jax
import jax.numpy as jnp

def _softmax(x, axis=-1):
    return jax.nn.softmax(x, axis=axis)
def _gelu(x):
    return jax.nn.gelu(x, approximate=True)
def _silu(x):
    return jax.nn.silu(x)
def _sigmoid(x):
    return jax.nn.sigmoid(x)
def _layernorm(x, axis=-1, eps=1e-5):
    m = jnp.mean(x, axis=axis, keepdims=True)
    v = jnp.var(x, axis=axis, keepdims=True)
    return (x - m) / jnp.sqrt(v + eps)
def _scatter_add(tgt, idx, src, axis=0):
    return tgt.at[idx].add(src)
def _segment_sum(src, seg, n):
    return jax.ops.segment_sum(src, seg, n)
class _Rng:
    def __init__(self, key):
        self._k = key
    def _next(self):
        self._k, sub = jax.random.split(self._k)
        return sub
    def normal(self, shape):
        return jax.random.normal(self._next(), shape, dtype=jnp.bfloat16)
    def randint(self, lo, hi, shape):
        return jax.random.randint(self._next(), shape, lo, hi, dtype=jnp.int32)
    def uniform(self, shape, lo=0.0, hi=1.0):
        return jax.random.uniform(self._next(), shape, jnp.bfloat16, lo, hi)
    def permutation(self, n):
        return jax.random.permutation(self._next(), n)


kernel_name = 'standalone__modern_conv_block_convnext_v2__vision'

def setup_inputs():
    _rng = _Rng(jax.random.key(int.from_bytes(__import__("os").urandom(4), "little")))
    _w = (lambda a: (lambda t: t.astype(jnp.bfloat16) if jnp.issubdtype(t.dtype, jnp.floating) else t)(jnp.asarray(a)))
    H = W = 512
    C = 96
    K = 3
    return {
        "x": _w((lambda *s: _rng.normal(s) * 0.05)(1, H, W, C)),
        "dw": _w((lambda *s: _rng.normal(s) * 0.05)(K, K, C)),
        "w1": _w((lambda *s: _rng.normal(s) * 0.05)(C, 4 * C)),
        "w2": _w((lambda *s: _rng.normal(s) * 0.05)(4 * C, C)),
        "grn_gamma": _w((lambda *s: _rng.normal(s) * 0.05)(4 * C)),
        "grn_beta": _w((lambda *s: _rng.normal(s) * 0.05)(4 * C)),
    }

def reference(x, dw, w1, w2, grn_gamma, grn_beta):
    B, H, W, C = x.shape
    K = dw.shape[0]
    pad = K // 2
    xp = jnp.pad(x, ((0,0),(pad,pad),(pad,pad),(0,0)))
    out = jnp.zeros_like(x)
    for i in range(K):
        for j in range(K):
            out = out + xp[:, i:i+H, j:j+W, :] * dw[i, j][None, None, None, :]
    h = _layernorm(out, axis=-1)
    h = jnp.einsum('bhwc,ce->bhwe', h, w1)
    h = _gelu(h)
    gx = jnp.sqrt((h * h).sum(axis=(1, 2), keepdims=True) + 1e-6)
    nx = gx / (gx.mean(axis=-1, keepdims=True) + 1e-6)
    h = grn_gamma * (h * nx) + grn_beta + h
    h = jnp.einsum('bhwe,ec->bhwc', h, w2)
    return x + h
```

```python
import functools
import math

import jax
import jax.numpy as jnp
import numpy as np
from jax import lax
import jax.experimental.pallas as pl
import jax.experimental.pallas.tpu as pltpu

F32 = jnp.float32
BF16 = jnp.bfloat16
U32 = jnp.uint32

_C0 = math.sqrt(2.0 / math.pi)
_C1 = 0.044715
_KS = (_C0 * _C1) ** (1.0 / 3.0)
_BS = _C0 / _KS


def _gelu_scaled(z):
    return z * (jnp.tanh(z * (z * z + _BS)) + 1.0)


def _kernel(x_hbm, dw_ref, w1_ref, w2t_ref, g_ref, b_ref, o_hbm,
            xbuf, obuf, sh, hs, lns, w1t, dcv, w2s, bias, acc, isem, osem,
            *, H, W, C, E, T, NB):
    G = C // 8
    NT = H // T
    xb32 = xbuf.bitcast(U32)

    def in1(b, slot):
        return pltpu.make_async_copy(x_hbm.at[pl.ds(b * T + 1, T)], xbuf.at[slot], isem.at[slot])

    def in1_last(slot):
        return pltpu.make_async_copy(x_hbm.at[pl.ds(H - T + 1, T - 1)], xbuf.at[slot, pl.ds(0, T - 1)], isem.at[slot])

    def start1(b):
        slot = b % NB
        @pl.when(b < NT - 1)
        def _():
            in1(b, slot).start()
        @pl.when(b == NT - 1)
        def _():
            in1_last(slot).start()

    def wait1(b):
        slot = b % NB
        @pl.when(b < NT - 1)
        def _():
            in1(b, slot).wait()
        @pl.when(b == NT - 1)
        def _():
            in1_last(slot).wait()
            xb32[slot, T - 1] = jnp.zeros((C // 2, W), U32)

    first = pltpu.make_async_copy(x_hbm.at[pl.ds(0, 1)], xbuf.at[NB - 1, pl.ds(1, 1)], isem.at[NB - 1])
    first.start()
    for b in range(NB - 1):
        in1(b, b).start()

    w1f = jnp.concatenate([w1_ref[...].astype(F32), jnp.zeros((128 - C, E), F32)], axis=0)
    w1t[...] = pltpu.bitcast(w1f.T.astype(BF16), U32)
    row = lax.broadcasted_iota(jnp.int32, (2 * C, 128), 0)
    col = lax.broadcasted_iota(jnp.int32, (2 * C, 128), 1)
    chan = (row >> 4) * 8 + (row & 7)
    r_out = (row >> 3) & 1
    blk = col >> 4
    p_in = jnp.where(blk >= 3, 1, 0)
    s_in = blk - 3 * p_in
    i_tap = 2 * p_in + ((col >> 3) & 1) - r_out
    same = ((col & 7) == (row & 7)) & (col < 96)
    d = jnp.zeros((2 * C, 128), F32)
    onehot = (col == chan)[:, :C]
    for i in range(3):
        dwi = dw_ref[i].astype(F32)
        for s in range(3):
            v = jnp.sum(jnp.where(onehot, dwi[s:s + 1, :], 0.0), axis=1, keepdims=True)
            d = jnp.where(same & (i_tap == i) & (s_in == s), v, d)
    dcv[...] = pltpu.bitcast(d.astype(BF16), U32)
    acc[...] = jnp.zeros_like(acc)

    lane = lax.broadcasted_iota(jnp.int32, (8, W), 1)

    def shift_pair(slot, r, dst):
        for g in range(G):
            m = jnp.concatenate([xb32[slot, r, pl.ds(4 * g, 4), :], xb32[slot, r + 1, pl.ds(4 * g, 4), :]], axis=0)
            sh[dst, g, pl.ds(0, 8), :] = jnp.where(lane == 0, jnp.uint32(0), pltpu.roll(m, 1, 1))
            sh[dst, g, pl.ds(8, 8), :] = m
            sh[dst, g, pl.ds(16, 8), :] = jnp.where(lane == W - 1, jnp.uint32(0), pltpu.roll(m, W - 1, 1))

    def conv_ln(p0, p1):
        o = [[], []]
        for g in range(G):
            rhs = pltpu.bitcast(jnp.concatenate([sh[p0, g], sh[p1, g]], axis=0), BF16)
            lhs = pltpu.bitcast(dcv[pl.ds(8 * g, 8), :], BF16)[:, :96]
            y = jnp.dot(lhs, rhs, preferred_element_type=F32)
            o[0].append(y[0:8])
            o[1].append(y[8:16])
        res = []
        for r in range(2):
            y = jnp.concatenate(o[r], axis=0)
            m = jnp.sum(y, axis=0, keepdims=True) * (1.0 / C)
            yc = y - m
            v = jnp.sum(yc * yc, axis=0, keepdims=True) * (1.0 / C)
            res.append((yc * (lax.rsqrt(v + 1e-5) * _KS)).astype(BF16))
        return res

    def mlp1(ln):
        z = jnp.dot(pltpu.bitcast(w1t[...], BF16)[:, :C], ln, preferred_element_type=F32)
        return _gelu_scaled(z)

    def sumsq(y):
        q = y * y
        t = q[:, 0:128]
        for k in range(1, W // 128):
            t = t + q[:, k * 128:(k + 1) * 128]
        return t

    xb32[NB - 1, 0] = jnp.zeros((C // 2, W), U32)
    first.wait()
    shift_pair(NB - 1, 0, 0)

    def body1(b, carry):
        @pl.when(b + NB - 1 < NT)
        def _():
            start1(b + NB - 1)
        wait1(b)
        slot = b % NB
        for u in range(T // 2):
            j = b * (T // 2) + u
            shift_pair(slot, 2 * u, (u + 1) & 1)
            ln0, ln1 = conv_ln(u & 1, (u + 1) & 1)
            lns[j] = pltpu.bitcast(ln1, U32)
            y0 = mlp1(ln0)
            hs[j] = pltpu.bitcast(y0.astype(BF16), U32)
            y1 = mlp1(ln1)
            acc[...] += sumsq(y0) + sumsq(y1)
        return carry

    lax.fori_loop(0, NT, body1, 0)

    def in2(b, slot):
        return pltpu.make_async_copy(x_hbm.at[pl.ds(b * T, T)], xbuf.at[slot], isem.at[slot])

    def out2(b, slot):
        return pltpu.make_async_copy(obuf.at[slot], o_hbm.at[pl.ds(b * T, T)], osem.at[slot])

    for b in range(NB - 1):
        in2(b, b).start()

    ss = jnp.sum(acc[...].T, axis=0, keepdims=True) * (1.0 / (4.0 * _KS * _KS))
    gx = jnp.sqrt(ss + 1e-6)
    nx = gx / (jnp.sum(gx, axis=1, keepdims=True) * (1.0 / E) + 1e-6)
    gam = g_ref[...].astype(F32).reshape(1, E)
    bet = b_ref[...].astype(F32).reshape(1, E)
    w2f = w2t_ref[...].astype(F32)
    w2s[...] = pltpu.bitcast((w2f * ((gam * nx + 1.0) * (0.5 / _KS))).astype(BF16), U32)
    bias[...] = jnp.broadcast_to(jnp.sum(w2f * bet, axis=1, keepdims=True), (C, 128))

    def mlp2(h, slot, r):
        y = jnp.dot(pltpu.bitcast(w2s[...], BF16), h, preferred_element_type=F32)
        bb = jnp.concatenate([bias[...]] * (W // 128), axis=1)
        obuf[slot, r] = (xbuf[slot, r].astype(F32) + bb + y).astype(BF16)

    def body2(b, carry):
        slot = b % NB
        @pl.when(b + NB - 1 < NT)
        def _():
            in2(b + NB - 1, (b + NB - 1) % NB).start()
        in2(b, slot).wait()
        @pl.when(b >= NB)
        def _():
            out2(b - NB, slot).wait()
        for u in range(T // 2):
            j = b * (T // 2) + u
            y1 = mlp1(pltpu.bitcast(lns[j], BF16)).astype(BF16)
            mlp2(pltpu.bitcast(hs[j], BF16), slot, 2 * u)
            mlp2(y1, slot, 2 * u + 1)
        out2(b, slot).start()
        return carry

    lax.fori_loop(0, NT, body2, 0)
    for b in range(NT - NB, NT):
        out2(b, b % NB).wait()


@jax.jit
def pallas_standalone__modern_conv_block_convnext_v2__vision_kernel(x, dw, w1, w2, grn_gamma, grn_beta):
    B, H, W, C = x.shape
    E = w1.shape[1]
    T, NB = 4, 4
    xt = x.reshape(H, W, C).transpose(0, 2, 1)
    vm = pl.BlockSpec(memory_space=pltpu.VMEM)
    out = pl.pallas_call(
        functools.partial(_kernel, H=H, W=W, C=C, E=E, T=T, NB=NB),
        out_shape=jax.ShapeDtypeStruct((H, C, W), x.dtype),
        in_specs=[pl.BlockSpec(memory_space=pl.ANY), vm, vm, vm, vm, vm],
        out_specs=pl.BlockSpec(memory_space=pl.ANY),
        scratch_shapes=[
            pltpu.VMEM((NB, T, C, W), BF16),
            pltpu.VMEM((NB, T, C, W), BF16),
            pltpu.VMEM((2, C // 8, 24, W), U32),
            pltpu.VMEM((H // 2, E // 2, W), U32),
            pltpu.VMEM((H // 2, C // 2, W), U32),
            pltpu.VMEM((E // 2, 128), U32),
            pltpu.VMEM((C, 128), U32),
            pltpu.VMEM((C // 2, E), U32),
            pltpu.VMEM((C, 128), F32),
            pltpu.VMEM((E, 128), F32),
            pltpu.SemaphoreType.DMA((NB,)),
            pltpu.SemaphoreType.DMA((NB,)),
        ],
        compiler_params=pltpu.CompilerParams(vmem_limit_bytes=128 * 2**20),
        name="convnext",
    )(xt, dw, w1, w2.T, grn_gamma, grn_beta)
    return out.transpose(0, 2, 1).reshape(B, H, W, C)
```

```python
import functools
import math

import jax
import jax.numpy as jnp
from jax import lax
import jax.experimental.pallas as pl
import jax.experimental.pallas.tpu as pltpu

F32 = jnp.float32
BF16 = jnp.bfloat16
U32 = jnp.uint32

_C0 = math.sqrt(2.0 / math.pi)
_C1 = 0.044715
_KS = (_C0 * _C1) ** (1.0 / 3.0)
_BS = _C0 / _KS

T = 8
R0, NR = 4, 3
KEPT = [r for r in range(T) if not R0 <= r < R0 + NR]
NX = 5
UB = 2
CH = 64
LEAD = 3
LN_ROW = (0, 1, 4, 5, 2, 3, 4, 5, 0, 1)
LN_CUR, LN_NEXT = (2, 3, 4), (0, 1, 5)

HEAD1 = "mmcmccc"
ORDER1 = HEAD1 + "mc" * (48 * UB - HEAD1.count("c"))
ORDER1 += "m" * (48 * UB - ORDER1.count("m"))
ORDER2 = "smsmrsmrssmrsmrssmrsmrssmrssmrsrs"
AFTER1 = (4, 4, 4, 4)
AFTER2 = (1, 5, 9)


def _gelu_scaled(z):
    return z * (jnp.tanh(z * (z * z + _BS)) + 1.0)


def _lanes(k):
    return pl.ds(128 * k, 128)


def _pack(v):
    return pltpu.bitcast(v.astype(BF16), U32)


def _unpack(v):
    return pltpu.bitcast(v, BF16)


def _after(step, result):
    return lambda v: jnp.where(step >= 0, v, result)


def _chain(gens):
    for g in gens:
        yield from g


def _kernel(x_hbm, dw_hbm, w1_hbm, w2t_hbm, gamma_hbm, beta_hbm, o_hbm,
            xbuf, hs, rss, cb0, cb1, cb2, cb3, lnb, sh, dcv, acc, w1t, dwc, w2s,
            w1_ref, w2t_ref, dw_ref, gamma_ref, beta_ref, isem, osem, wsem):
    H, C, W = x_hbm.shape
    E = w1_hbm.shape[1]
    G, NT, KW, NK = C // 8, H // T, W // 128, E // 128
    hs, lnb = hs.bitcast(BF16), lnb.bitcast(BF16)
    cbuf = (cb0, cb1, cb2, cb3)
    lane = lax.broadcasted_iota(jnp.int32, (8, 128), 1)
    sub = lax.broadcasted_iota(jnp.int32, (8, 128), 0)

    def slot_of(v):
        return (v - NT) % NX

    def ahead(slot, n):
        return slot + n - jnp.where(slot + n >= NX, NX, 0)

    def x_copy(v, slot):
        row = jnp.where(v < NT, jnp.minimum(v * T + LEAD, H - T), jnp.maximum(2 * NT - 1 - v, 0) * T)
        return pltpu.make_async_copy(x_hbm.at[pl.ds(row, T)], xbuf.at[pl.ds(slot * T, T)], isem.at[slot])

    def o_copy(b, slot):
        return pltpu.make_async_copy(
            xbuf.at[pl.ds(slot * T, T)], o_hbm.at[pl.ds((NT - 1 - b) * T, T)], osem.at[slot])

    top = slot_of(NX - 1) * T
    head = pltpu.make_async_copy(x_hbm.at[pl.ds(0, LEAD)], xbuf.at[pl.ds(top + 1, LEAD)], osem.at[0])
    small = [pltpu.make_async_copy(src, dst, wsem.at[i]) for i, (src, dst) in enumerate((
        (dw_hbm, dw_ref), (w1_hbm, w1_ref), (w2t_hbm, w2t_ref), (gamma_hbm, gamma_ref), (beta_hbm, beta_ref)))]
    for c in (*small[:2], head, *[x_copy(v, slot_of(v)) for v in range(UB)]):
        c.start()
    for c in small[:2]:
        c.wait()
    xbuf[top] = jnp.zeros((C, W), BF16)
    xbuf[NX * T] = jnp.zeros((C, W), BF16)

    w1f = w1_ref[...].astype(F32)
    w1f = w1f - jnp.sum(w1f, axis=0, keepdims=True) * (1.0 / C)
    w1t[...] = _pack(jnp.concatenate([w1f, jnp.zeros((128 - C, E), F32)], axis=0).T)

    dwt = jnp.concatenate(
        [jnp.pad(dw_ref[i].astype(F32), ((0, 5), (0, 128 - C))) for i in range(3)]
        + [jnp.zeros((104, 128), F32)], axis=0).T[:C]
    dwc[...] = dwt
    for g in range(G):
        halves = []
        for r in range(2):
            d = jnp.zeros((8, 128), F32)
            for i in range(3):
                for s in range(3):
                    pair, row = divmod(i + r, 2)
                    d = jnp.where(lane - sub == ((pair * 3 + s) * 2 + row) * 8,
                                  dwt[8 * g:8 * g + 8, 8 * i + s:8 * i + s + 1], d)
            halves.append(d)
        dcv[pl.ds(8 * g, 8), :] = _pack(jnp.concatenate(halves, axis=0))
    acc[...] = jnp.zeros_like(acc)

    def shifted(r, g, k, par):
        def fetch(kk):
            v = pltpu.bitcast(xbuf[pl.ds(r, 2), pl.ds(8 * g, 8), _lanes(kk)].reshape(16, 128), U32)
            sh[g, pl.ds(24 * par + 8, 8), _lanes(kk)] = v
            return v
        zero = jnp.zeros((8, 128), U32)
        mid = fetch(0) if k == 0 else sh[g, pl.ds(24 * par + 8, 8), _lanes(k)]
        prv = zero if k == 0 else sh[g, pl.ds(24 * par + 8, 8), _lanes(k - 1)]
        nxt = zero if k == KW - 1 else fetch(k + 1)
        lft = pltpu.roll(jnp.where(lane == 127, prv, mid), 1, 1)
        rgt = pltpu.roll(jnp.where(lane == 0, nxt, mid), 127, 1)
        sh[g, pl.ds(24 * par, 8), _lanes(k)] = lft
        sh[g, pl.ds(24 * par + 16, 8), _lanes(k)] = rgt
        return jnp.concatenate([lft, mid, rgt], axis=0)

    def fold4(a, b):
        return jnp.where(sub < 4, a, b) + pltpu.roll(jnp.where(sub < 4, b, a), 4, 0)

    def fold1(a, b):
        t = jnp.where((sub & 2) == 0, a + pltpu.roll(a, 6, 0), b + pltpu.roll(b, 2, 0))
        return t + pltpu.roll(t, 1, 0)

    pending = []

    def normalize(scales, step, b, row, k, after):
        i = 4 * (row % 2) + 1 + 2 * (k % 2)
        scale = after(scales)[i:i + 1]
        if R0 <= row < R0 + NR:
            rss[b, pl.ds((row - R0) * KW + k, 1), :] = scale
        y = cbuf[k][row % 2 + jnp.minimum(step, 0)]
        lnb[pl.ds(LN_ROW[row], 1), :, _lanes(k)] = (y * scale)[None].astype(BF16)

    def conv_steps(step, b, u, r):
        par = u % 2
        for k in range(KW):
            s1, s2 = [None, None], [None, None]
            for g in range(G):
                above = sh[g, pl.ds(24 * (1 - par), 24), _lanes(k)]
                rhs = _unpack(jnp.concatenate([above, shifted(r, g, k, par)], axis=0))
                y = jnp.dot(_unpack(dcv[pl.ds(8 * g, 8), :])[:, :96], rhs, preferred_element_type=F32)
                for q in range(2):
                    yq = y[8 * q:8 * q + 8]
                    cbuf[k][q, pl.ds(8 * g, 8), :] = yq
                    s1[q] = yq if g == 0 else s1[q] + yq
                    s2[q] = yq * yq if g == 0 else s2[q] + yq * yq
                if g == G - 1 and k % 2 == 0:
                    t1, t2 = fold4(*s1), fold4(*s2)
                elif g == G - 1:
                    m = fold1(t1, fold4(*s1)) * (1.0 / (C * _KS))
                    v = fold1(t2, fold4(*s2)) * (1.0 / (C * _KS * _KS)) - m * m
                    scales = lax.rsqrt(jnp.maximum(v, 0.0) + 1e-5 / (_KS * _KS))
                    pending.extend(functools.partial(normalize, scales, step, b, 2 * u + q, kk)
                                   for kk in (k - 1, k) for q in range(2))
                if g % 4 == 3:
                    yield

    def mlp_steps(step, b, u):
        for k0 in range(0, KW, 2):
            for e in range(0, E, CH):
                rhs = jnp.concatenate(
                    [lnb[LN_ROW[2 * u + q], :, pl.ds(128 * k0, 256)] for q in range(2)], axis=1)
                lhs = _unpack(w1t[pl.ds(e // 2, CH // 2), :])[:, :C]
                y = _gelu_scaled(jnp.dot(lhs, rhs, preferred_element_type=F32))
                t = acc[pl.ds(e, CH), :]
                for i in range(4):
                    yi = y[:, 128 * i:128 * (i + 1)]
                    row = 2 * u + i // 2
                    if row in KEPT:
                        hs[pl.ds(b * len(KEPT) + KEPT.index(row), 1), pl.ds(e, CH), _lanes(k0 + i % 2)] = (
                            yi[None].astype(BF16))
                    t = t + yi * yi
                acc[pl.ds(e, CH), :] = t
                for i, f in zip(AFTER1, pending):
                    f(_after(step, t[8 * i:8 * i + 8]))
                pending.clear()
                yield

    head.wait()
    for k in range(KW):
        for g in range(G):
            shifted(top, g, k, 1)
    for _ in conv_steps(0, 0, 0, top + 2):
        pass
    for f in pending:
        f(lambda v: v)
    pending.clear()
    for v in range(UB):
        x_copy(v, slot_of(v)).wait()
    for c in (*[x_copy(v, slot_of(v)) for v in range(UB, NX - UB)], *small[2:]):
        c.start()

    def body1(step, slot):
        blocks = [step * UB + i for i in range(UB)]
        for i, b in enumerate(blocks):
            x_copy(b + NX - UB, ahead(slot, i + NX - UB)).start()
        mlp, conv = [], []
        for i, b in enumerate(blocks):
            for u in range(T // 2):
                r = ahead(slot, i) * T + jnp.minimum(2 * u + jnp.where(b == NT - 1, LEAD, 0), T - 1)
                mlp.append(mlp_steps(step, b, u))
                conv.append(conv_steps(step, b, u + 1, r))
        work = {"m": _chain(mlp), "c": _chain(conv)}
        for ch in ORDER1:
            next(work[ch])
        assert all(next(g, 1) == 1 for g in work.values()) and not pending
        for i, b in enumerate(blocks):
            x_copy(b + UB, ahead(slot, i + UB)).wait()
        return ahead(slot, UB)

    lax.fori_loop(0, NT // UB, body1, slot_of(0))
    for v in range(NT + NX - UB, NT + NX - 1):
        x_copy(v, slot_of(v)).start()

    for c in small[2:]:
        c.wait()
    gx = jnp.sqrt(jnp.sum(acc[...].T, axis=0, keepdims=True) * (0.25 / (_KS * _KS)) + 1e-6)
    nx = gx / (jnp.sum(gx, axis=1, keepdims=True) * (1.0 / E) + 1e-6)
    gamma = gamma_ref[...].astype(F32).reshape(1, E)
    beta = beta_ref[...].astype(F32).reshape(1, E)
    w2f = w2t_ref[...].astype(F32)
    w2n = w2f * ((gamma * nx + 1.0) * (0.5 / _KS))
    for k in range(NK):
        w2s[:, _lanes(k)] = _pack(w2n[:, 128 * k:128 * (k + 1)])
    acc[pl.ds(0, C), :] = jnp.broadcast_to(jnp.sum(w2f * beta, axis=1, keepdims=True), (C, 128))

    for i in range(3):
        for s in range(3):
            t = jnp.broadcast_to(dwc[:, 8 * i + s:8 * i + s + 1], (C, 128))
            sh[:, pl.ds(8 * i, 8), _lanes(s)] = pltpu.bitcast(t, U32).reshape(G, 8, 128)

    def tap(i, s, g):
        return pltpu.bitcast(sh[g, pl.ds(8 * i, 8), _lanes(s)], F32)

    def reconv_steps(blk, slot):
        zero = jnp.zeros((8, 128), F32)
        ys = None
        for g in range(G):
            xs = [xbuf[slot * T + R0 - 1 + r, pl.ds(8 * g, 8), :].astype(F32) for r in range(NR + 2)]
            cols = []
            for k in range(KW):
                after = yield
                xk = [after(v[:, 128 * k:128 * (k + 1)]) for v in xs]
                cols.append([[xk[r] * tap(0, s, g) + xk[r + 1] * tap(1, s, g) + xk[r + 2] * tap(2, s, g)
                              for s in range(3)] for r in range(NR)])
            prev, ys = ys, []
            for k in range(KW):
                for r in range(NR):
                    prv = zero if k == 0 else cols[k - 1][r][0]
                    nxt = zero if k == KW - 1 else cols[k + 1][r][2]
                    y = (cols[k][r][1] + pltpu.roll(jnp.where(lane == 127, prv, cols[k][r][0]), 1, 1)
                         + pltpu.roll(jnp.where(lane == 0, nxt, cols[k][r][2]), 127, 1))
                    ys.append(y * rss[blk, pl.ds(r * KW + k, 1), :])
                    if g % 2:
                        lnb[pl.ds(LN_NEXT[r], 1), pl.ds(8 * g - 8, 16), _lanes(k)] = (
                            jnp.concatenate([prev[k * NR + r], ys[-1]], axis=0)[None].astype(BF16))
        yield

    def rebuild(r, kt):
        lhs = jnp.concatenate([w1t[pl.ds(64 * kt + 8 * i, 8), :] for i in reversed(range(8))], axis=0)
        y = _gelu_scaled(jnp.dot(_unpack(lhs)[:, :C], lnb[LN_CUR[r]], preferred_element_type=F32))
        return jnp.concatenate([y[16 * i:16 * i + 16] for i in reversed(range(8))], axis=0).astype(BF16)

    def project(h, kt, part, row):
        y = jnp.dot(_unpack(w2s[:, _lanes(kt)]), h, preferred_element_type=F32)
        if kt == 0:
            t = xbuf[row].astype(F32) + jnp.concatenate([acc[pl.ds(0, C), :]] * KW, axis=1) + y
        else:
            t = jnp.concatenate([c[part] for c in cbuf], axis=1) + y
        if kt < NK - 1:
            for k in range(KW):
                cbuf[k][part] = t[:, 128 * k:128 * (k + 1)]
        else:
            xbuf[row] = t.astype(BF16)
        return y

    def body2(b, slot):
        stored = o_copy(jnp.maximum(b - 1, 0), ahead(slot, NX - 1))
        fetch = x_copy(NT + b + NX - 1, ahead(slot, NX - 1))
        ready = x_copy(NT + b + 2, ahead(slot, 2))
        conv = reconv_steps(jnp.maximum(NT - 2 - b, 0), ahead(slot, 1))
        next(conv)
        left = G * KW
        rebuilt = []
        count = {"m": 0, "s": 0, "r": 0}
        for ch in ORDER2:
            u, kt = divmod(count[ch], NK)
            count[ch] += 1
            if ch == "m":
                rebuilt.append(rebuild(u, kt))
                continue
            if ch == "s":
                h = hs[(NT - 1 - b) * len(KEPT) + u, pl.ds(128 * kt, 128), :]
                y = project(h, kt, 0, slot * T + KEPT[u])
            else:
                y = project(rebuilt.pop(0), kt, 1, slot * T + R0 + u)
            for i in AFTER2[:left]:
                left -= 1
                conv.send(_after(b, y[8 * i:8 * i + 8, :128]))
        assert left == 0 and count == {"m": NR * NK, "r": NR * NK, "s": len(KEPT) * NK}
        for r in range(NR):
            lnb[LN_CUR[r]] = lnb[LN_NEXT[r]]
        o_copy(b, slot).start()
        pl.when(b > 0)(stored.wait)
        pl.when(b + NX - 1 < NT)(fetch.start)
        pl.when(b + 2 < NT)(ready.wait)
        return ahead(slot, 1)

    lax.fori_loop(0, NT, body2, slot_of(NT))
    o_copy(NT - 1, slot_of(2 * NT - 1)).wait()


@jax.jit
def pallas_standalone__modern_conv_block_convnext_v2__vision_kernel(
    x: jax.Array,
    dw: jax.Array,
    w1: jax.Array,
    w2: jax.Array,
    grn_gamma: jax.Array,
    grn_beta: jax.Array,
):
    B, H, W, C = x.shape
    E = w1.shape[1]
    assert (B, W, C, E, dw.shape) == (1, 512, 96, 384, (3, 3, C)) and H % (T * UB) == 0 and H >= T * NX
    out = pl.pallas_call(
        _kernel,
        out_shape=jax.ShapeDtypeStruct((H, C, W), x.dtype),
        in_specs=[pl.BlockSpec(memory_space=pl.ANY)] * 6,
        out_specs=pl.BlockSpec(memory_space=pl.ANY),
        scratch_shapes=[
            pltpu.VMEM((NX * T + 1, C, W), BF16),
            pltpu.VMEM((H // T * len(KEPT), E // 2, W), U32),
            pltpu.VMEM((H // T, 16, 128), F32),
            *[pltpu.VMEM((2, C, 128), F32)] * 4,
            pltpu.VMEM((2 * NR, C // 2, W), U32),
            pltpu.VMEM((C // 8, 48, W), U32),
            pltpu.VMEM((C, 128), U32),
            pltpu.VMEM((E, 128), F32),
            pltpu.VMEM((E // 2, 128), U32),
            pltpu.VMEM((C, 128), F32),
            pltpu.VMEM((C // 2, E), U32),
            *[pltpu.VMEM(v.shape, v.dtype) for v in (w1, w1, dw, grn_gamma, grn_beta)],
            pltpu.SemaphoreType.DMA((NX,)),
            pltpu.SemaphoreType.DMA((NX,)),
            pltpu.SemaphoreType.DMA((5,)),
        ],
        compiler_params=pltpu.CompilerParams(vmem_limit_bytes=128 * 2**20, disable_bounds_checks=True),
        name="convnext",
    )(x.reshape(H, W, C).transpose(0, 2, 1), dw, w1, w2.T, grn_gamma, grn_beta)
    return out.transpose(0, 2, 1).reshape(B, H, W, C)
```

```python
import functools
import math

import jax
import jax.numpy as jnp
from jax import lax
import jax.experimental.pallas as pl
import jax.experimental.pallas.tpu as pltpu

F32 = jnp.float32
BF16 = jnp.bfloat16
U32 = jnp.uint32

_C0 = math.sqrt(2.0 / math.pi)
_C1 = 0.044715
_KS = (_C0 * _C1) ** (1.0 / 3.0)
_BS = _C0 / _KS

T = 8
R0, NR = 4, 3
KEPT = [r for r in range(T) if not R0 <= r < R0 + NR]
NX = 5
UB = 2
CH = 64
LEAD = 3
LN_ROW = (0, 1, 4, 5, 2, 3, 4, 5, 0, 1)
LN_CUR, LN_NEXT = (2, 3, 4), (0, 1, 5)

HEAD1 = "mmcmcccmc"
ORDER1 = HEAD1 + "mc" * (48 * UB - HEAD1.count("c"))
ORDER1 += "m" * (48 * UB - ORDER1.count("m"))
ORDER2 = "msmrsmrssmrssmrssmrsmrssmrsmrssrs"
AFTER1 = (3, 7, 7, 5)
AFTER2 = (3, 4, 9)


def _gelu_scaled(z):
    return z * (jnp.tanh(z * (z * z + _BS)) + 1.0)


def _lanes(k):
    return pl.ds(128 * k, 128)


def _pack(v):
    return pltpu.bitcast(v.astype(BF16), U32)


def _unpack(v):
    return pltpu.bitcast(v, BF16)


def _after(step, result):
    return lambda v: jnp.where(step >= 0, v, result)


def _chain(gens):
    for g in gens:
        yield from g


def _kernel(x_hbm, dw_hbm, w1_hbm, w2t_hbm, gamma_hbm, beta_hbm, o_hbm,
            xbuf, hs, rss, cb0, cb1, cb2, cb3, lnb, sh, dcv, acc, w1t, dwc, w2s,
            w1_ref, w2t_ref, dw_ref, gamma_ref, beta_ref, isem, osem, wsem):
    H, C, W = x_hbm.shape
    E = w1_hbm.shape[1]
    G, NT, KW, NK = C // 8, H // T, W // 128, E // 128
    hs, lnb = hs.bitcast(BF16), lnb.bitcast(BF16)
    cbuf = (cb0, cb1, cb2, cb3)
    lane = lax.broadcasted_iota(jnp.int32, (8, 128), 1)
    sub = lax.broadcasted_iota(jnp.int32, (8, 128), 0)

    def slot_of(v):
        return (v - NT) % NX

    def ahead(slot, n):
        return slot + n - jnp.where(slot + n >= NX, NX, 0)

    def x_copy(v, slot):
        row = jnp.where(v < NT, jnp.minimum(v * T + LEAD, H - T), jnp.maximum(2 * NT - 1 - v, 0) * T)
        return pltpu.make_async_copy(x_hbm.at[pl.ds(row, T)], xbuf.at[pl.ds(slot * T, T)], isem.at[slot])

    def o_copy(b, slot):
        return pltpu.make_async_copy(
            xbuf.at[pl.ds(slot * T, T)], o_hbm.at[pl.ds((NT - 1 - b) * T, T)], osem.at[slot])

    top = slot_of(NX - 1) * T
    head = pltpu.make_async_copy(x_hbm.at[pl.ds(0, LEAD)], xbuf.at[pl.ds(top + 1, LEAD)], osem.at[0])
    small = [pltpu.make_async_copy(src, dst, wsem.at[i]) for i, (src, dst) in enumerate((
        (dw_hbm, dw_ref), (w1_hbm, w1_ref), (w2t_hbm, w2t_ref), (gamma_hbm, gamma_ref), (beta_hbm, beta_ref)))]
    for c in (*small[:2], head, *[x_copy(v, slot_of(v)) for v in range(UB)]):
        c.start()
    for c in small[:2]:
        c.wait()
    xbuf[top] = jnp.zeros((C, W), BF16)
    xbuf[NX * T] = jnp.zeros((C, W), BF16)

    w1f = w1_ref[...].astype(F32) * _KS
    for _ in range(4):
        w1f = w1f - jnp.sum(w1f.astype(BF16).astype(F32), axis=0, keepdims=True) * (1.0 / C)
    w1t[...] = _pack(jnp.concatenate([w1f, jnp.zeros((128 - C, E), F32)], axis=0).T)

    dwt = jnp.concatenate(
        [jnp.pad(dw_ref[i].astype(F32), ((0, 5), (0, 128 - C))) for i in range(3)]
        + [jnp.zeros((104, 128), F32)], axis=0).T[:C]
    dwc[...] = dwt
    for g in range(G):
        halves = []
        for r in range(2):
            d = jnp.zeros((8, 128), F32)
            for i in range(3):
                for s in range(3):
                    pair, row = divmod(i + r, 2)
                    d = jnp.where(lane - sub == ((pair * 3 + s) * 2 + row) * 8,
                                  dwt[8 * g:8 * g + 8, 8 * i + s:8 * i + s + 1], d)
            halves.append(d)
        dcv[pl.ds(8 * g, 8), :] = _pack(jnp.concatenate(halves, axis=0))
    acc[...] = jnp.zeros_like(acc)

    def shifted(r, g, k, par):
        def fetch(kk):
            v = pltpu.bitcast(xbuf[pl.ds(r, 2), pl.ds(8 * g, 8), _lanes(kk)].reshape(16, 128), U32)
            sh[g, pl.ds(24 * par + 8, 8), _lanes(kk)] = v
            return v
        zero = jnp.zeros((8, 128), U32)
        mid = fetch(0) if k == 0 else sh[g, pl.ds(24 * par + 8, 8), _lanes(k)]
        prv = zero if k == 0 else sh[g, pl.ds(24 * par + 8, 8), _lanes(k - 1)]
        nxt = zero if k == KW - 1 else fetch(k + 1)
        lft = pltpu.roll(jnp.where(lane == 127, prv, mid), 1, 1)
        rgt = pltpu.roll(jnp.where(lane == 0, nxt, mid), 127, 1)
        sh[g, pl.ds(24 * par, 8), _lanes(k)] = lft
        sh[g, pl.ds(24 * par + 16, 8), _lanes(k)] = rgt
        return jnp.concatenate([lft, mid, rgt], axis=0)

    def fold4(a, b):
        return jnp.where(sub < 4, a, b) + pltpu.roll(jnp.where(sub < 4, b, a), 4, 0)

    def fold1(a, b):
        t = jnp.where((sub & 2) == 0, a + pltpu.roll(a, 6, 0), b + pltpu.roll(b, 2, 0))
        return t + pltpu.roll(t, 1, 0)

    pending = []

    def normalize(scales, step, b, row, k, after):
        i = 4 * (row % 2) + 1 + 2 * (k % 2)
        scale = after(scales)[i:i + 1]
        if R0 <= row < R0 + NR:
            rss[b, pl.ds((row - R0) * KW + k, 1), :] = scale
        y = cbuf[k][row % 2 + jnp.minimum(step, 0)]
        lnb[pl.ds(LN_ROW[row], 1), :, _lanes(k)] = (y * scale)[None].astype(BF16)

    def conv_steps(step, b, u, r):
        par = u % 2
        for k in range(KW):
            s1, s2 = [None, None], [None, None]
            for g in range(G):
                above = sh[g, pl.ds(24 * (1 - par), 24), _lanes(k)]
                rhs = _unpack(jnp.concatenate([above, shifted(r, g, k, par)], axis=0))
                y = jnp.dot(_unpack(dcv[pl.ds(8 * g, 8), :])[:, :96], rhs, preferred_element_type=F32)
                for q in range(2):
                    yq = y[8 * q:8 * q + 8]
                    cbuf[k][q, pl.ds(8 * g, 8), :] = yq
                    s1[q] = yq if g == 0 else s1[q] + yq
                    s2[q] = yq * yq if g == 0 else s2[q] + yq * yq
                if g == G - 1 and k % 2 == 0:
                    t1, t2 = fold4(*s1), fold4(*s2)
                elif g == G - 1:
                    m = fold1(t1, fold4(*s1)) * (1.0 / C)
                    v = fold1(t2, fold4(*s2)) * (1.0 / C) - m * m
                    scales = lax.rsqrt(jnp.maximum(v, 0.0) + 1e-5)
                    pending.extend(functools.partial(normalize, scales, step, b, 2 * u + q, kk)
                                   for kk in (k - 1, k) for q in range(2))
                if g % 4 == 3:
                    yield

    def mlp_steps(step, b, u):
        for k0 in range(0, KW, 2):
            for e in range(0, E, CH):
                rhs = jnp.concatenate(
                    [lnb[LN_ROW[2 * u + q], :, pl.ds(128 * k0, 256)] for q in range(2)], axis=1)
                lhs = _unpack(w1t[pl.ds(e // 2, CH // 2), :])[:, :C]
                y = _gelu_scaled(jnp.dot(lhs, rhs, preferred_element_type=F32))
                t = acc[pl.ds(e, CH), :]
                for i in range(4):
                    yi = y[:, 128 * i:128 * (i + 1)]
                    row = 2 * u + i // 2
                    if row in KEPT:
                        hs[pl.ds(b * len(KEPT) + KEPT.index(row), 1), pl.ds(e, CH), _lanes(k0 + i % 2)] = (
                            yi[None].astype(BF16))
                    t = t + yi * yi
                acc[pl.ds(e, CH), :] = t
                for i, f in zip(AFTER1, pending):
                    f(_after(step, t[8 * i:8 * i + 8]))
                pending.clear()
                yield

    head.wait()
    for k in range(KW):
        for g in range(G):
            shifted(top, g, k, 1)
    for _ in conv_steps(0, 0, 0, top + 2):
        pass
    for f in pending:
        f(lambda v: v)
    pending.clear()
    for v in range(UB):
        x_copy(v, slot_of(v)).wait()
    for c in (*[x_copy(v, slot_of(v)) for v in range(UB, NX - UB)], *small[2:]):
        c.start()

    def body1(step, slot):
        blocks = [step * UB + i for i in range(UB)]
        for i, b in enumerate(blocks):
            x_copy(b + NX - UB, ahead(slot, i + NX - UB)).start()
        mlp, conv = [], []
        for i, b in enumerate(blocks):
            for u in range(T // 2):
                r = ahead(slot, i) * T + jnp.minimum(2 * u + jnp.where(b == NT - 1, LEAD, 0), T - 1)
                mlp.append(mlp_steps(step, b, u))
                conv.append(conv_steps(step, b, u + 1, r))
        work = {"m": _chain(mlp), "c": _chain(conv)}
        for ch in ORDER1:
            next(work[ch])
        assert all(next(g, 1) == 1 for g in work.values()) and not pending
        for i, b in enumerate(blocks):
            x_copy(b + UB, ahead(slot, i + UB)).wait()
        return ahead(slot, UB)

    lax.fori_loop(0, NT // UB, body1, slot_of(0))
    for v in range(NT + NX - UB, NT + NX - 1):
        x_copy(v, slot_of(v)).start()

    for c in small[2:]:
        c.wait()
    gx = jnp.sqrt(jnp.sum(acc[...].T, axis=0, keepdims=True) * (0.25 / (_KS * _KS)) + 1e-6)
    nx = gx / (jnp.sum(gx, axis=1, keepdims=True) * (1.0 / E) + 1e-6)
    gamma = gamma_ref[...].astype(F32).reshape(1, E)
    beta = beta_ref[...].astype(F32).reshape(1, E)
    w2f = w2t_ref[...].astype(F32)
    w2n = w2f * ((gamma * nx + 1.0) * (0.5 / _KS))
    for k in range(NK):
        w2s[:, _lanes(k)] = _pack(w2n[:, 128 * k:128 * (k + 1)])
    acc[pl.ds(0, C), :] = jnp.broadcast_to(jnp.sum(w2f * beta, axis=1, keepdims=True), (C, 128))

    for i in range(3):
        for s in range(3):
            t = jnp.broadcast_to(dwc[:, 8 * i + s:8 * i + s + 1], (C, 128))
            sh[:, pl.ds(8 * i, 8), _lanes(s)] = pltpu.bitcast(t, U32).reshape(G, 8, 128)

    def tap(i, s, g):
        return pltpu.bitcast(sh[g, pl.ds(8 * i, 8), _lanes(s)], F32)

    def reconv_steps(blk, slot):
        zero = jnp.zeros((8, 128), F32)
        ys = None
        for g in range(G):
            xs = [xbuf[slot * T + R0 - 1 + r, pl.ds(8 * g, 8), :].astype(F32) for r in range(NR + 2)]
            cols = []
            for k in range(KW):
                after = yield
                xk = [after(v[:, 128 * k:128 * (k + 1)]) for v in xs]
                cols.append([[xk[r] * tap(0, s, g) + xk[r + 1] * tap(1, s, g) + xk[r + 2] * tap(2, s, g)
                              for s in range(3)] for r in range(NR)])
            prev, ys = ys, []
            for k in range(KW):
                for r in range(NR):
                    prv = zero if k == 0 else cols[k - 1][r][0]
                    nxt = zero if k == KW - 1 else cols[k + 1][r][2]
                    y = (cols[k][r][1] + pltpu.roll(jnp.where(lane == 127, prv, cols[k][r][0]), 1, 1)
                         + pltpu.roll(jnp.where(lane == 0, nxt, cols[k][r][2]), 127, 1))
                    ys.append(y * rss[blk, pl.ds(r * KW + k, 1), :])
                    if g % 2:
                        lnb[pl.ds(LN_NEXT[r], 1), pl.ds(8 * g - 8, 16), _lanes(k)] = (
                            jnp.concatenate([prev[k * NR + r], ys[-1]], axis=0)[None].astype(BF16))
        yield

    def rebuild(r, kt):
        lhs = jnp.concatenate([w1t[pl.ds(64 * kt + 8 * i, 8), :] for i in reversed(range(8))], axis=0)
        y = _gelu_scaled(jnp.dot(_unpack(lhs)[:, :C], lnb[LN_CUR[r]], preferred_element_type=F32))
        return jnp.concatenate([y[16 * i:16 * i + 16] for i in reversed(range(8))], axis=0).astype(BF16)

    def project(h, kt, part, row):
        y = jnp.dot(_unpack(w2s[:, _lanes(kt)]), h, preferred_element_type=F32)
        if kt == 0:
            t = xbuf[row].astype(F32) + jnp.concatenate([acc[pl.ds(0, C), :]] * KW, axis=1) + y
        else:
            t = jnp.concatenate([c[part] for c in cbuf], axis=1) + y
        if kt < NK - 1:
            for k in range(KW):
                cbuf[k][part] = t[:, 128 * k:128 * (k + 1)]
        else:
            xbuf[row] = t.astype(BF16)
        return y

    def body2(b, slot):
        stored = o_copy(jnp.maximum(b - 1, 0), ahead(slot, NX - 1))
        fetch = x_copy(NT + b + NX - 1, ahead(slot, NX - 1))
        ready = x_copy(NT + b + 2, ahead(slot, 2))
        conv = reconv_steps(jnp.maximum(NT - 2 - b, 0), ahead(slot, 1))
        next(conv)
        left = G * KW
        rebuilt = []
        count = {"m": 0, "s": 0, "r": 0}
        for ch in ORDER2:
            u, kt = divmod(count[ch], NK)
            count[ch] += 1
            if ch == "m":
                rebuilt.append(rebuild(u, kt))
                continue
            if ch == "s":
                h = hs[(NT - 1 - b) * len(KEPT) + u, pl.ds(128 * kt, 128), :]
                y = project(h, kt, 0, slot * T + KEPT[u])
            else:
                y = project(rebuilt.pop(0), kt, 1, slot * T + R0 + u)
            for i in AFTER2[:left]:
                left -= 1
                conv.send(_after(b, y[8 * i:8 * i + 8, :128]))
        assert left == 0 and count == {"m": NR * NK, "r": NR * NK, "s": len(KEPT) * NK}
        for r in range(NR):
            lnb[LN_CUR[r]] = lnb[LN_NEXT[r]]
        o_copy(b, slot).start()
        pl.when(b > 0)(stored.wait)
        pl.when(b + NX - 1 < NT)(fetch.start)
        pl.when(b + 2 < NT)(ready.wait)
        return ahead(slot, 1)

    lax.fori_loop(0, NT, body2, slot_of(NT))
    o_copy(NT - 1, slot_of(2 * NT - 1)).wait()


@jax.jit
def pallas_standalone__modern_conv_block_convnext_v2__vision_kernel(
    x: jax.Array,
    dw: jax.Array,
    w1: jax.Array,
    w2: jax.Array,
    grn_gamma: jax.Array,
    grn_beta: jax.Array,
):
    B, H, W, C = x.shape
    E = w1.shape[1]
    assert (B, W, C, E, dw.shape) == (1, 512, 96, 384, (3, 3, C)) and H % (T * UB) == 0 and H >= T * NX
    out = pl.pallas_call(
        _kernel,
        out_shape=jax.ShapeDtypeStruct((H, C, W), x.dtype),
        in_specs=[pl.BlockSpec(memory_space=pl.ANY)] * 6,
        out_specs=pl.BlockSpec(memory_space=pl.ANY),
        scratch_shapes=[
            pltpu.VMEM((NX * T + 1, C, W), BF16),
            pltpu.VMEM((H // T * len(KEPT), E // 2, W), U32),
            pltpu.VMEM((H // T, 16, 128), F32),
            *[pltpu.VMEM((2, C, 128), F32)] * 4,
            pltpu.VMEM((2 * NR, C // 2, W), U32),
            pltpu.VMEM((C // 8, 48, W), U32),
            pltpu.VMEM((C, 128), U32),
            pltpu.VMEM((E, 128), F32),
            pltpu.VMEM((E // 2, 128), U32),
            pltpu.VMEM((C, 128), F32),
            pltpu.VMEM((C // 2, E), U32),
            *[pltpu.VMEM(v.shape, v.dtype) for v in (w1, w1, dw, grn_gamma, grn_beta)],
            pltpu.SemaphoreType.DMA((NX,)),
            pltpu.SemaphoreType.DMA((NX,)),
            pltpu.SemaphoreType.DMA((5,)),
        ],
        compiler_params=pltpu.CompilerParams(vmem_limit_bytes=128 * 2**20, disable_bounds_checks=True),
        name="convnext",
    )(x.reshape(H, W, C).transpose(0, 2, 1), dw, w1, w2.T, grn_gamma, grn_beta)
    return out.transpose(0, 2, 1).reshape(B, H, W, C)
```
